```python
import os as _os
_os.environ.setdefault("JAX_PLATFORMS", "cpu")
import jax
import jax.numpy as jnp

def _softmax(x, axis=-1):
    return jax.nn.softmax(x, axis=axis)
def _gelu(x):
    return jax.nn.gelu(x, approximate=True)
def _silu(x):
    return jax.nn.silu(x)
def _sigmoid(x):
    return jax.nn.sigmoid(x)
def _layernorm(x, axis=-1, eps=1e-5):
    m = jnp.mean(x, axis=axis, keepdims=True)
    v = jnp.var(x, axis=axis, keepdims=True)
    return (x - m) / jnp.sqrt(v + eps)
def _scatter_add(tgt, idx, src, axis=0):
    return tgt.at[idx].add(src)
def _segment_sum(src, seg, n):
    return jax.ops.segment_sum(src, seg, n)
class _Rng:
    def __init__(self, key):
        self._k = key
    def _next(self):
        self._k, sub = jax.random.split(self._k)
        return sub
    def normal(self, shape):
        return jax.random.normal(self._next(), shape, dtype=jnp.bfloat16)
    def randint(self, lo, hi, shape):
        return jax.random.randint(self._next(), shape, lo, hi, dtype=jnp.int32)
    def uniform(self, shape, lo=0.0, hi=1.0):
        return jax.random.uniform(self._next(), shape, jnp.bfloat16, lo, hi)
    def permutation(self, n):
        return jax.random.permutation(self._next(), n)


kernel_name = 'interleave_layers__sliding_block_cached__mixer_channel_mlp__decode'

def setup_inputs():
    _rng = _Rng(jax.random.key(int.from_bytes(__import__("os").urandom(4), "little")))
    _w = (lambda a: (lambda t: t.astype(jnp.bfloat16) if jnp.issubdtype(t.dtype, jnp.floating) else t)(jnp.asarray(a)))
    def _A_setup():
        B, Sq, D = 8, 1, 1024
        Hq, Hkv, Sk, Dh = 32, 4, 4096, 128
        assert Hq % Hkv == 0, (Hq, Hkv)
        return {
            "x": _w((lambda *s: _rng.normal(s) * 0.05)(B, Sq, D)),
            "k_cache": _w((lambda *s: _rng.normal(s) * 1.6)(B, Hkv, Sk, Dh)),
            "v_cache": _w((lambda *s: _rng.normal(s) * 0.8)(B, Hkv, Sk, Dh)),
            "wq": _w((lambda *s: _rng.normal(s) * 1.6)(D, Hq * Dh) * (D ** -0.5)),
            "wo": _w((lambda *s: _rng.normal(s) * 0.8)(Hq * Dh, D) * ((Hq * Dh) ** -0.5)),
        }
    _A_in = _A_setup()

    def _B_setup():
        B, S, D, F = 8, 1, 1024, 3584
        return {
            "x": _w((lambda *s: _rng.normal(s) * 0.05)(B, S, D)),
            "w1": _w((lambda *s: _rng.normal(s) * 0.4)(D, F) * (D ** -0.5)),
            "b1": _w((lambda *s: _rng.normal(s) * 0.4)(F)),
            "w2": _w((lambda *s: _rng.normal(s) * 0.4)(F, D) * (F ** -0.5)),
            "b2": _w((lambda *s: _rng.normal(s) * 0.1)(D)),
        }
    _B_in = _B_setup()

    return {
        "A_x": _A_in["x"],
        "A_k_cache": _A_in["k_cache"],
        "A_v_cache": _A_in["v_cache"],
        "A_wq": _A_in["wq"],
        "A_wo": _A_in["wo"],
        "B_x": _B_in["x"],
        "B_w1": _B_in["w1"],
        "B_b1": _B_in["b1"],
        "B_w2": _B_in["w2"],
        "B_b2": _B_in["b2"],
    }

def reference(A_x, A_k_cache, A_v_cache, A_wq, A_wo, B_x, B_w1, B_b1, B_w2, B_b2):
    def _A_ref(x, k_cache, v_cache, wq, wo):
        B, Sq, D = x.shape
        Hq, Dh = 32, 128
        Hkv, Sk = k_cache.shape[1], k_cache.shape[2]
        W = min(4096, max(256, Sk // 4))
        rep = Hq // Hkv
        q = (lambda x, *d: x.transpose(*d))((x @ wq).reshape(B, Sq, Hq, Dh), 0, 2, 1, 3)
        k = jnp.repeat(k_cache[:, :, Sk - W:, :], rep, axis=1)
        v = jnp.repeat(v_cache[:, :, Sk - W:, :], rep, axis=1)
        scores = jnp.einsum("bhqd,bhkd->bhqk", q, k) * (Dh ** -0.5)
        p = _softmax(scores, axis=-1)
        o = jnp.einsum("bhqk,bhkd->bhqd", p, v)
        return (lambda x, *d: x.transpose(*d))(o, 0, 2, 1, 3).reshape(B, Sq, Hq * Dh) @ wo

    def _B_ref(x, w1, b1, w2, b2):
        y = _layernorm(x, axis=-1)
        h = _gelu(jnp.einsum("bsd,df->bsf", y, w1) + b1)
        return jnp.einsum("bsf,fd->bsd", h, w2) + b2

    x = A_x
    x = x + _A_ref(_layernorm(x, axis=-1), A_k_cache, A_v_cache, A_wq, A_wo)
    x = x + _B_ref(_layernorm(x, axis=-1), B_w1, B_b1, B_w2, B_b2)
    x = x + _A_ref(_layernorm(x, axis=-1), A_k_cache, A_v_cache, A_wq, A_wo)
    x = x + _B_ref(_layernorm(x, axis=-1), B_w1, B_b1, B_w2, B_b2)
    return x
```

```python
import functools

import jax
import jax.numpy as jnp
import jax.experimental.pallas as pl
import jax.experimental.pallas.tpu as pltpu

_EPS = 1e-5
_BF16 = jnp.bfloat16
_F32 = jnp.float32


def _ln_stats(x):
    m = jnp.mean(x, axis=-1, keepdims=True)
    xc = x - m
    v = jnp.mean(xc * xc, axis=-1, keepdims=True)
    return m, xc, jax.lax.rsqrt(v + _EPS)


def _gelu_tanh(x):
    c = 0.7978845608028654
    return 0.5 * x * (1.0 + jnp.tanh(c * (x + 0.044715 * (x * x * x))))


def _dot(a, b):
    return jnp.dot(a, b, preferred_element_type=_F32)


def _chunks(total, sizes):
    out, r = [], 0
    for s in sizes:
        out.append((r, s))
        r += s
    assert r == total, (r, total)
    return out


def _kernel(x_hbm, k_hbm, v_hbm, wq_hbm, wo_hbm, w1_hbm, b1_hbm, w2_hbm, b2_hbm,
            o_ref,
            x_s, b1_s, b2_s, k_s, v_s, kt_s,
            wq_r, wo_r, w1_r, w2_r, wq_t, wo_t, w1_t, w2_t,
            q_s, o_s, sems,
            *, B, D, Hq, Hkv, Sk, Dh, W, F):
    rep = Hq // Hkv
    scale = Dh ** -0.5
    G = rep * Dh

    wq_ch = _chunks(D, (512, 512))
    kv_ch = _chunks(B, (4, 4))
    wo_ch = _chunks(Hq * Dh, (2048, 2048))
    w1_ch = _chunks(D, (512, 512))
    w2_ch = _chunks(F, (1536, 1024, 512, 256, 256))

    n_sem = [1]

    def mk(src, dst):
        c = pltpu.make_async_copy(src, dst, sems.at[n_sem[0]])
        n_sem[0] += 1
        return c

    small = [pltpu.make_async_copy(x_hbm, x_s, sems.at[0]),
             pltpu.make_async_copy(b1_hbm, b1_s, sems.at[0]),
             pltpu.make_async_copy(b2_hbm, b2_s, sems.at[0])]
    wq_cp = [mk(wq_hbm.at[pl.ds(r, n), :], wq_r.at[pl.ds(r, n), :]) for r, n in wq_ch]
    k_cp = [mk(k_hbm.at[pl.ds(r, n), :, pl.ds(Sk - W, W), :], k_s.at[pl.ds(r, n)])
            for r, n in kv_ch]
    v_cp = [mk(v_hbm.at[pl.ds(r, n), :, pl.ds(Sk - W, W), :], v_s.at[pl.ds(r, n)])
            for r, n in kv_ch]
    wo_cp = [mk(wo_hbm.at[pl.ds(r, n), :], wo_r.at[pl.ds(r, n), :]) for r, n in wo_ch]
    w1_cp = [mk(w1_hbm.at[pl.ds(r, n), :], w1_r.at[pl.ds(r, n), :]) for r, n in w1_ch]
    w2_cp = [mk(w2_hbm.at[pl.ds(r, n), :], w2_r.at[pl.ds(r, n), :]) for r, n in w2_ch]

    for c in small + wq_cp + k_cp + v_cp + wo_cp + w1_cp + w2_cp:
        c.start()
    for c in small:
        c.wait()

    x = x_s[...].astype(_F32)
    b1 = b1_s[...].astype(_F32).reshape(1, F)
    b2 = b2_s[...].astype(_F32).reshape(1, D)

    def stream_matmul(a, w_r, w_t, chunks, copies, kblk, nblk):
        N = w_r.shape[1]
        accs = [None] * (N // nblk)
        for (r0, n), cp in zip(chunks, copies):
            cp.wait()
            for kk in range(r0, r0 + n, kblk):
                a_k = a[:, kk:kk + kblk]
                for j in range(N // nblk):
                    w = w_r[kk:kk + kblk, j * nblk:(j + 1) * nblk]
                    w_t[kk // 2:(kk + kblk) // 2, j * nblk:(j + 1) * nblk] = (
                        pltpu.bitcast(w, jnp.uint32))
                    d = _dot(a_k, w)
                    accs[j] = d if accs[j] is None else accs[j] + d
        return jnp.concatenate(accs, axis=1)

    def wt(w_t, k0, k1, n0, n1):
        return pltpu.bitcast(w_t[k0 // 2:k1 // 2, n0:n1], _BF16)

    def with_ones(x32):
        return jnp.concatenate([x32, jnp.ones_like(x32)], axis=0).astype(_BF16)

    def put_q(q, h0):
        for h in range(q.shape[1] // Dh):
            q_s[(h0 + h) * B:(h0 + h + 1) * B, :] = q[:, h * Dh:(h + 1) * Dh]

    def scores(b, g):
        qg = q_s[pl.ds(g * rep * B + b, rep, stride=B), :].astype(_BF16)
        s = _dot(qg, pltpu.bitcast(kt_s[b, g], _BF16))
        m = jnp.max(s, axis=-1, keepdims=True)
        e = jnp.exp(s - m)
        l = jnp.sum(e, axis=-1, keepdims=True)
        return e.astype(_BF16), l

    def pv(b, g, e, l):
        o = _dot(e, v_s[b, g]) / l
        o_s[pl.ds(g * rep * B + b, rep, stride=B), :] = o

    def get_o(h0, h1):
        return jnp.concatenate(
            [o_s[h * B:(h + 1) * B, :] for h in range(h0, h1)], axis=1).astype(_BF16)

    def ln2_coeffs(x):
        m1, xc, r1 = _ln_stats(x)
        m2, _, r2 = _ln_stats(xc * r1)
        return r1 * r2, (m1 * r1 + m2) * r2

    m, _, r = _ln_stats(x)
    qq = stream_matmul(with_ones(x), wq_r, wq_t, wq_ch, wq_cp, 128, 1024)
    csq = qq[B:]
    put_q((qq[:B] - m * csq) * (r * scale), 0)
    el = {}
    for (r0, n), cp in zip(kv_ch, k_cp):
        cp.wait()
        for b in range(r0, r0 + n):
            for g in range(Hkv):
                kt_s[b, g] = pltpu.bitcast(k_s[b, g].T, jnp.uint32)
                el[b, g] = scores(b, g)
    for (r0, n), cp in zip(kv_ch, v_cp):
        cp.wait()
        for b in range(r0, r0 + n):
            for g in range(Hkv):
                pv(b, g, *el[b, g])
    x = x + stream_matmul(get_o(0, Hq), wo_r, wo_t, wo_ch, wo_cp, 128, 1024)
    x = x.astype(_BF16).astype(_F32)
    a, c = ln2_coeffs(x)
    hh = stream_matmul(with_ones(x), w1_r, w1_t, w1_ch, w1_cp, 128, 896)
    cs1 = hh[B:]
    h = _gelu_tanh(a * hh[:B] - c * cs1 + b1).astype(_BF16)
    x = x + stream_matmul(h, w2_r, w2_t, w2_ch, w2_cp, 128, 1024) + b2

    xb = x.astype(_BF16)
    x = xb.astype(_F32)
    m, _, r = _ln_stats(x)
    rs = r * scale
    for g in range(Hkv):
        qg = _dot(xb, wt(wq_t, 0, D, g * G, (g + 1) * G))
        put_q((qg - m * csq[:, g * G:(g + 1) * G]) * rs, g * rep)
    for g in range(Hkv):
        for b in range(B):
            el[b, g] = scores(b, g)
    for g in range(Hkv):
        for b in range(B):
            pv(b, g, *el[b, g])
    acc = x
    for g in range(Hkv):
        acc = acc + _dot(get_o(g * rep, (g + 1) * rep), wt(wo_t, g * G, (g + 1) * G, 0, D))
    xb = acc.astype(_BF16)
    x = xb.astype(_F32)
    a, c = ln2_coeffs(x)
    hp = None
    for j in range(D // 128):
        d = _dot(xb[:, j * 128:(j + 1) * 128], wt(w1_t, j * 128, (j + 1) * 128, 0, F))
        hp = d if hp is None else hp + d
    h = _gelu_tanh(a * hp - c * cs1 + b1).astype(_BF16)
    acc = x + b2
    for f0 in range(0, F, 512):
        acc = acc + _dot(h[:, f0:f0 + 512], wt(w2_t, f0, f0 + 512, 0, D))

    o_ref[...] = acc.astype(o_ref.dtype)


@jax.jit
def pallas_interleave_layers__sliding_block_cached__mixer_channel_mlp__decode_kernel(
    A_x: jax.Array,
    A_k_cache: jax.Array,
    A_v_cache: jax.Array,
    A_wq: jax.Array,
    A_wo: jax.Array,
    B_x: jax.Array,
    B_w1: jax.Array,
    B_b1: jax.Array,
    B_w2: jax.Array,
    B_b2: jax.Array,
):
    del B_x
    B, Sq, D = A_x.shape
    assert Sq == 1
    _, Hkv, Sk, Dh = A_k_cache.shape
    Hq = A_wq.shape[1] // Dh
    F = B_w1.shape[1]
    W = min(4096, max(256, Sk // 4))

    kernel = functools.partial(
        _kernel, B=B, D=D, Hq=Hq, Hkv=Hkv, Sk=Sk, Dh=Dh, W=W, F=F)
    any_spec = pl.BlockSpec(memory_space=pl.ANY)
    u32 = jnp.uint32
    scratch = [
        pltpu.VMEM((B, D), _BF16),
        pltpu.VMEM((F,), _BF16),
        pltpu.VMEM((D,), _BF16),
        pltpu.VMEM((B, Hkv, W, Dh), _BF16),
        pltpu.VMEM((B, Hkv, W, Dh), _BF16),
        pltpu.VMEM((B, Hkv, Dh // 2, W), u32),
        pltpu.VMEM((D, Hq * Dh), _BF16),
        pltpu.VMEM((Hq * Dh, D), _BF16),
        pltpu.VMEM((D, F), _BF16),
        pltpu.VMEM((F, D), _BF16),
        pltpu.VMEM((D // 2, Hq * Dh), u32),
        pltpu.VMEM((Hq * Dh // 2, D), u32),
        pltpu.VMEM((D // 2, F), u32),
        pltpu.VMEM((F // 2, D), u32),
        pltpu.VMEM((Hq * B, Dh), _F32),
        pltpu.VMEM((Hq * B, Dh), _F32),
        pltpu.SemaphoreType.DMA((16,)),
    ]
    out = pl.pallas_call(
        kernel,
        out_shape=jax.ShapeDtypeStruct((B, D), A_x.dtype),
        in_specs=[any_spec] * 9,
        out_specs=pl.BlockSpec(memory_space=pltpu.VMEM),
        scratch_shapes=scratch,
        compiler_params=pltpu.CompilerParams(vmem_limit_bytes=110 * 1024 * 1024),
    )(A_x.reshape(B, D), A_k_cache, A_v_cache, A_wq, A_wo, B_w1, B_b1, B_w2, B_b2)
    return out.reshape(B, Sq, D)
```

```python
import functools

import jax
import jax.numpy as jnp
import jax.experimental.pallas as pl
import jax.experimental.pallas.tpu as pltpu

_EPS = 1e-5
_BF16 = jnp.bfloat16
_F32 = jnp.float32

R1, RC, RB, RA = 512, 1536, 1920, 2560
LATE_R = 1
QSCHED = "|||0123|4a|4b5a|5b6a|6b7"
F_, D_ = 3584, 1024
W2_RECTS = [(R1, RC, 0, 512), (RC, RB, 0, 640), (RB, RA, 0, 768), (RA, F_, 0, 896),
            (R1, RC, 512, D_), (RC, RB, 640, D_), (RB, RA, 768, D_), (RA, F_, 896, D_)]
W2K = 2
NSEM = 64


def _ln_stats(x):
    m = jnp.mean(x, axis=-1, keepdims=True)
    xc = x - m
    v = jnp.mean(xc * xc, axis=-1, keepdims=True)
    return m, xc, jax.lax.rsqrt(v + _EPS)


def _gelu_tanh(x):
    c = 0.7978845608028654
    return 0.5 * x * (1.0 + jnp.tanh(c * (x + 0.044715 * (x * x * x))))


def _dot(a, b):
    return jnp.dot(a, b, preferred_element_type=_F32)


def _kernel(*refs, **kw):
    pl.run_scoped(lambda sems: _body(*refs, sems, **kw),
                  pltpu.SemaphoreType.DMA((NSEM,)))


def _body(x_hbm, k_hbm, v_hbm, wq_hbm, wo_hbm, w1_hbm, b1_hbm, w2_hbm, b2_hbm,
          o_ref,
          x_s, b1_s, b2_s, k_s, v_s, kt_s,
          wq_r, wo_r, w1_r, w2_r,
          wq_t, wo_t, w1_t, w2_t,
          a_s, acc_s, q_s, o_s, p0, p1, p2, p3, p4, p5, p6, p7, sems,
          *, B, D, Hq, Hkv, Sk, Dh, W, F):
    rep = Hq // Hkv
    scale = Dh ** -0.5
    G = rep * Dh
    NJ = D // 128
    HD = Hq * Dh

    sem_base = [1]

    class Stream:
        def __init__(self, hbm, buf, rows, chunk):
            self.hbm, self.buf, self.chunk = hbm, buf, chunk
            self.n = rows // chunk
            self.base = sem_base[0]
            sem_base[0] += self.n

        def copy(self, i):
            r = i * self.chunk
            if not isinstance(i, int):
                r = pl.multiple_of(r, self.chunk)
            return pltpu.make_async_copy(
                self.hbm.at[pl.ds(r, self.chunk), :],
                self.buf.at[pl.ds(r, self.chunk), :],
                sems.at[self.base + i])

    def kv_copy(b, which):
        hbm, buf = (k_hbm, k_s) if which == 0 else (v_hbm, v_s)
        return pltpu.make_async_copy(
            hbm.at[b, :, pl.ds(Sk - W, W), :], buf.at[b],
            sems.at[kv_base + 2 * b + which])

    small = [pltpu.make_async_copy(x_hbm, x_s, sems.at[0]),
             pltpu.make_async_copy(b1_hbm, b1_s, sems.at[0]),
             pltpu.make_async_copy(b2_hbm, b2_s, sems.at[0])]
    wq_st = Stream(wq_hbm, wq_r, D, 128)
    kv_base = sem_base[0]
    sem_base[0] += 2 * B
    wo_st = Stream(wo_hbm, wo_r, HD, 512)
    w1_st = Stream(w1_hbm, w1_r, D, 128)
    w2_st = Stream(w2_hbm, w2_r, R1, 512)
    w2_rects = [t + (p,) for t, p in zip(W2_RECTS, (p0, p1, p2, p3, p4, p5, p6, p7))]
    def parse(s):
        out, i = [], 0
        while i < len(s):
            j = int(s[i]); i += 1
            gs = list(range(Hkv))
            if i < len(s) and s[i] in "ab":
                gs = gs[:Hkv // 2] if s[i] == "a" else gs[Hkv // 2:]
                i += 1
            out.append((j, gs))
        return out
    qs = [parse(s) for s in QSCHED.split("|")]
    w2_cp = []
    for (r0, r1, c0, c1, dst) in w2_rects:
        w2_cp.append(pltpu.make_async_copy(
            w2_hbm.at[pl.ds(r0, r1 - r0), pl.ds(c0, c1 - c0)], dst,
            sems.at[sem_base[0]]))
        sem_base[0] += 1
    assert sem_base[0] <= NSEM

    wq_st.copy(0).start()
    for c in small:
        c.start()
    for i in range(1, wq_st.n):
        wq_st.copy(i).start()
    for b in range(B):
        kv_copy(b, 0).start()
        kv_copy(b, 1).start()
    for st in (wo_st, w1_st, w2_st):
        for i in range(st.n):
            st.copy(i).start()
    for c in w2_cp:
        c.start()
    for c in small:
        c.wait()

    x = x_s[...].astype(_F32)
    b1 = b1_s[...].astype(_F32).reshape(1, F)
    b2 = b2_s[...].astype(_F32).reshape(1, D)

    def stream_matmul(a, st, w_t, nblk):
        N = st.buf.shape[1]
        kpc = st.chunk // 128
        for kt in range(st.n * kpc):
            a_s[kt] = a[:, kt * 128:(kt + 1) * 128]
        acc_s[:, 0:N] = jnp.zeros((2 * B, N), _F32)

        def body(i, carry):
            st.copy(i).wait()
            for u in range(kpc):
                kt = i * kpc + u
                a_k = a_s[kt]
                r = pl.multiple_of(kt * 128, 128)
                rh = pl.multiple_of(kt * 64, 64)
                for j in range(N // nblk):
                    w = st.buf[pl.ds(r, 128), j * nblk:(j + 1) * nblk]
                    w_t[pl.ds(rh, 64), j * nblk:(j + 1) * nblk] = (
                        pltpu.bitcast(w, jnp.uint32))
                    acc_s[:, j * nblk:(j + 1) * nblk] += _dot(a_k, w)
            return carry

        jax.lax.fori_loop(0, st.n, body, 0)
        return acc_s[:, 0:N]

    def wt(w_t, k0, k1, n0, n1):
        return pltpu.bitcast(w_t[k0 // 2:k1 // 2, n0:n1], _BF16)

    def with_ones(x32):
        return jnp.concatenate([x32, jnp.ones_like(x32)], axis=0).astype(_BF16)

    def put_q(q, h0):
        for h in range(q.shape[1] // Dh):
            q_s[(h0 + h) * B:(h0 + h + 1) * B, :] = q[:, h * Dh:(h + 1) * Dh]

    def scores(b, g, c=None):
        qg = q_s[pl.ds(g * rep * B + b, rep, stride=B), :].astype(_BF16)
        s = _dot(qg, pltpu.bitcast(kt_s[b, g], _BF16))
        m = jnp.max(s, axis=-1, keepdims=True)
        if c is None:
            e = jnp.exp(s - m)
        else:
            e = jnp.exp2((s - m) * c)
        l = jnp.sum(e, axis=-1, keepdims=True)
        return e.astype(_BF16), l

    def pv(b, g, e, l):
        o = _dot(e, v_s[b, g]) / l
        o_s[pl.ds(g * rep * B + b, rep, stride=B), :] = o

    def get_o(h0, h1):
        return jnp.concatenate(
            [o_s[h * B:(h + 1) * B, :] for h in range(h0, h1)], axis=1)

    def ln2_coeffs(x):
        m1, xc, r1 = _ln_stats(x)
        m2, _, r2 = _ln_stats(xc * r1)
        return r1 * r2, (m1 * r1 + m2) * r2

    m, _, r = _ln_stats(x)
    qq = stream_matmul(with_ones(x), wq_st, wq_t, 1024)
    csq = qq[B:]
    put_q((qq[:B] - m * csq) * (r * scale), 0)
    el = {}

    def attn1(b, carry):
        kv_copy(b, 0).wait()
        for g in range(Hkv):
            kt_s[b, g] = pltpu.bitcast(k_s[b, g].T, jnp.uint32)
        for g in range(Hkv):
            el[g] = scores(b, g)
        kv_copy(b, 1).wait()
        for g in range(Hkv):
            pv(b, g, *el[g])
        return carry

    jax.lax.fori_loop(0, B, attn1, 0)
    x = x + stream_matmul(with_ones(get_o(0, Hq)), wo_st, wo_t, 1024)[:B]
    x = x.astype(_BF16).astype(_F32)
    a, c = ln2_coeffs(x)
    hh = stream_matmul(with_ones(x), w1_st, w1_t, 896)
    cs1 = hh[B:]
    h32 = _gelu_tanh(a * hh[:B] - c * cs1 + b1)
    h = h32.astype(_BF16)
    xb2 = x + b2 + stream_matmul(with_ones(h32[:, :R1]), w2_st, w2_t, 1024)[:B]

    acc = [xb2[:, j * 128:(j + 1) * 128] for j in range(NJ)]
    xbs = [None] * NJ
    qpre = [None] * Hkv
    left = [F - R1] * NJ

    def q_part(j, gs):
        for g in gs:
            d = _dot(xbs[j], wt(wq_t, j * 128, (j + 1) * 128, g * G, (g + 1) * G))
            qpre[g] = d if qpre[g] is None else qpre[g] + d

    for (r0, r1, c0, c1, buf), cp, qlist in zip(w2_rects, w2_cp, qs):
        cp.wait()
        if c1 - c0 == 128:
            j = c0 // 128
            acc[j] = acc[j] + _dot(h[:, r0:r1], buf[...])
        else:
            for kk in range(r0, r1, 128):
                w = buf[kk - r0:kk - r0 + 128, :]
                w2_t[kk // 2:(kk + 128) // 2, c0:c1] = pltpu.bitcast(w, jnp.uint32)
                d = _dot(h[:, kk:kk + 128], w)
                for j in range(c0 // 128, c1 // 128):
                    acc[j] = acc[j] + d[:, j * 128 - c0:(j + 1) * 128 - c0]
        for j in range(c0 // 128, c1 // 128):
            left[j] -= r1 - r0
            if left[j] == 0:
                xbs[j] = acc[j].astype(_BF16)
        for j, gs in qlist:
            q_part(j, gs)

    x = jnp.concatenate(xbs, axis=1).astype(_F32)
    m, _, r = _ln_stats(x)
    if LATE_R:
        rs = r * (scale * 1.4426950408889634)
        for g in range(Hkv):
            put_q(qpre[g] - m * csq[:, g * G:(g + 1) * G], g * rep)
        for g in range(Hkv):
            for b in range(B):
                el[b, g] = scores(b, g, rs[b:b + 1, :])
    else:
        rs = r * scale
        for g in range(Hkv):
            put_q((qpre[g] - m * csq[:, g * G:(g + 1) * G]) * rs, g * rep)
        for g in range(Hkv):
            for b in range(B):
                el[b, g] = scores(b, g)
    for g in range(Hkv):
        for b in range(B):
            pv(b, g, *el[b, g])
    acc = x
    for g in range(Hkv):
        acc = acc + _dot(get_o(g * rep, (g + 1) * rep).astype(_BF16),
                         wt(wo_t, g * G, (g + 1) * G, 0, D))
    xb = acc.astype(_BF16)
    x = xb.astype(_F32)
    a, c = ln2_coeffs(x)
    hp = None
    for j in range(D // 128):
        d = _dot(xb[:, j * 128:(j + 1) * 128], wt(w1_t, j * 128, (j + 1) * 128, 0, F))
        hp = d if hp is None else hp + d
    h = _gelu_tanh(a * hp - c * cs1 + b1).astype(_BF16)
    acc = x + b2
    for f0 in range(0, RA, 128 * W2K):
        f1 = min(f0 + 128 * W2K, RA)
        acc = acc + _dot(h[:, f0:f1], wt(w2_t, f0, f1, 0, D))
    h_tail = h[:, RA:]
    acc = acc + jnp.concatenate(
        [_dot(h_tail, wt(w2_t, RA, F, 0, D - 128)), _dot(h_tail, p7[...])], axis=1)

    o_ref[...] = acc.astype(o_ref.dtype)


@jax.jit
def pallas_interleave_layers__sliding_block_cached__mixer_channel_mlp__decode_kernel(
    A_x: jax.Array,
    A_k_cache: jax.Array,
    A_v_cache: jax.Array,
    A_wq: jax.Array,
    A_wo: jax.Array,
    B_x: jax.Array,
    B_w1: jax.Array,
    B_b1: jax.Array,
    B_w2: jax.Array,
    B_b2: jax.Array,
):
    del B_x
    B, Sq, D = A_x.shape
    assert Sq == 1
    _, Hkv, Sk, Dh = A_k_cache.shape
    Hq = A_wq.shape[1] // Dh
    F = B_w1.shape[1]
    W = min(4096, max(256, Sk // 4))

    kernel = functools.partial(
        _kernel, B=B, D=D, Hq=Hq, Hkv=Hkv, Sk=Sk, Dh=Dh, W=W, F=F)
    any_spec = pl.BlockSpec(memory_space=pl.ANY)
    u32 = jnp.uint32
    scratch = [
        pltpu.VMEM((B, D), _BF16),
        pltpu.VMEM((F,), _BF16),
        pltpu.VMEM((D,), _BF16),
        pltpu.VMEM((B, Hkv, W, Dh), _BF16),
        pltpu.VMEM((B, Hkv, W, Dh), _BF16),
        pltpu.VMEM((B, Hkv, Dh // 2, W), u32),
        pltpu.VMEM((D, Hq * Dh), _BF16),
        pltpu.VMEM((Hq * Dh, D), _BF16),
        pltpu.VMEM((D, F), _BF16),
        pltpu.VMEM((R1, D), _BF16),
        pltpu.VMEM((D // 2, Hq * Dh), u32),
        pltpu.VMEM((Hq * Dh // 2, D), u32),
        pltpu.VMEM((D // 2, F), u32),
        pltpu.VMEM((F // 2, D), u32),
        pltpu.VMEM((Hq * Dh // 128, 2 * B, 128), _BF16),
        pltpu.VMEM((2 * B, Hq * Dh), _F32),
        pltpu.VMEM((Hq * B, Dh), _F32),
        pltpu.VMEM((Hq * B, Dh), _F32),
    ] + [pltpu.VMEM((r1 - r0, c1 - c0), _BF16) for (r0, r1, c0, c1) in W2_RECTS]
    out = pl.pallas_call(
        kernel,
        out_shape=jax.ShapeDtypeStruct((B, D), A_x.dtype),
        in_specs=[any_spec] * 9,
        out_specs=pl.BlockSpec(memory_space=pltpu.VMEM),
        scratch_shapes=scratch,
        compiler_params=pltpu.CompilerParams(vmem_limit_bytes=110 * 1024 * 1024),
    )(A_x.reshape(B, D), A_k_cache, A_v_cache, A_wq, A_wo, B_w1, B_b1, B_w2, B_b2)
    return out.reshape(B, Sq, D)
```

```python
import functools

import jax
import jax.numpy as jnp
import jax.experimental.pallas as pl
import jax.experimental.pallas.tpu as pltpu

_EPS = 1e-5
_LOG2E = 1.4426950408889634
_BF16 = jnp.bfloat16
_F32 = jnp.float32

_R1, _RC, _RB, _RA = 512, 1536, 1920, 2560
_LO, _HI, _ALL = (0, 1), (2, 3), (0, 1, 2, 3)
_QSCHED = (
    (), (), (),
    ((0, _ALL), (1, _ALL), (2, _ALL), (3, _ALL)),
    ((4, _LO),),
    ((4, _HI), (5, _LO)),
    ((5, _HI), (6, _LO)),
    ((6, _HI), (7, _ALL)),
)
_NSEM = 50


def _w2_rects(F, D):
    left = [(_R1, _RC, 0, 512), (_RC, _RB, 0, 640), (_RB, _RA, 0, 768), (_RA, F, 0, 896)]
    return left + [(r0, r1, c1, D) for (r0, r1, _, c1) in left]


def _ln_stats(x):
    m = jnp.mean(x, axis=-1, keepdims=True)
    xc = x - m
    v = jnp.mean(xc * xc, axis=-1, keepdims=True)
    return m, xc, jax.lax.rsqrt(v + _EPS)


def _ln2_coeffs(x):
    m1, xc, r1 = _ln_stats(x)
    m2, _, r2 = _ln_stats(xc * r1)
    return r1 * r2, (m1 * r1 + m2) * r2


def _gelu_tanh(x):
    c = 0.7978845608028654
    return 0.5 * x * (1.0 + jnp.tanh(c * (x + 0.044715 * (x * x * x))))


def _dot(a, b):
    return jnp.dot(a, b, preferred_element_type=_F32)


def _with_ones(x32):
    return jnp.concatenate([x32, jnp.ones_like(x32)], axis=0).astype(_BF16)


def _kernel(*refs, **kw):
    pl.run_scoped(lambda sems: _body(*refs, sems, **kw),
                  pltpu.SemaphoreType.DMA((_NSEM,)))


def _body(x_hbm, k_hbm, v_hbm, wq_hbm, wo_hbm, w1_hbm, b1_hbm, w2_hbm, b2_hbm,
          o_ref,
          x_s, b1_s, b2_s, k_s, v_s, kt_s,
          wq_r, wo_r, w1_r, w2_r,
          wq_t, wo_t, w1_t, w2_t,
          a_s, acc_s, q_s, o_s, p0, p1, p2, p3, p4, p5, p6, p7, sems,
          *, B, D, Hq, Hkv, Sk, Dh, W, F):
    rep = Hq // Hkv
    scale = Dh ** -0.5
    G = rep * Dh
    NJ = D // 128
    HD = Hq * Dh

    next_sem = [1]

    def take_sems(n):
        base = next_sem[0]
        next_sem[0] += n
        return base

    class Stream:
        def __init__(self, hbm, buf, rows, chunk):
            self.hbm, self.buf, self.chunk = hbm, buf, chunk
            self.n = rows // chunk
            self.base = take_sems(self.n)

        def copy(self, i):
            r = i * self.chunk
            if not isinstance(i, int):
                r = pl.multiple_of(r, self.chunk)
            return pltpu.make_async_copy(
                self.hbm.at[pl.ds(r, self.chunk), :],
                self.buf.at[pl.ds(r, self.chunk), :],
                sems.at[self.base + i])

    small = [pltpu.make_async_copy(x_hbm, x_s, sems.at[0]),
             pltpu.make_async_copy(b1_hbm, b1_s, sems.at[0]),
             pltpu.make_async_copy(b2_hbm, b2_s, sems.at[0])]
    wq_st = Stream(wq_hbm, wq_r, D, 128)
    kv_base = take_sems(2 * B)
    wo_st = Stream(wo_hbm, wo_r, HD, 512)
    w1_st = Stream(w1_hbm, w1_r, D, 128)
    w2_st = Stream(w2_hbm, w2_r, _R1, 512)
    rects = _w2_rects(F, D)
    rect_bufs = (p0, p1, p2, p3, p4, p5, p6, p7)
    rect_cp = [
        pltpu.make_async_copy(
            w2_hbm.at[pl.ds(r0, r1 - r0), pl.ds(c0, c1 - c0)], buf,
            sems.at[take_sems(1)])
        for (r0, r1, c0, c1), buf in zip(rects, rect_bufs)]
    assert next_sem[0] <= _NSEM

    def kv_copy(b, which):
        hbm, buf = (k_hbm, k_s) if which == 0 else (v_hbm, v_s)
        return pltpu.make_async_copy(
            hbm.at[b, :, pl.ds(Sk - W, W), :], buf.at[b],
            sems.at[kv_base + 2 * b + which])

    wq_st.copy(0).start()
    for c in small:
        c.start()
    for i in range(1, wq_st.n):
        wq_st.copy(i).start()
    for b in range(B):
        kv_copy(b, 0).start()
        kv_copy(b, 1).start()
    for st in (wo_st, w1_st, w2_st):
        for i in range(st.n):
            st.copy(i).start()
    for c in rect_cp:
        c.start()

    q_s[Hq * B:, :] = jnp.zeros((B, Dh), _F32)
    o_s[Hq * B:, :] = jnp.zeros((B, Dh), _F32)

    for c in small:
        c.wait()
    x = x_s[...].astype(_F32)
    b1 = b1_s[...].astype(_F32).reshape(1, F)
    b2 = b2_s[...].astype(_F32).reshape(1, D)

    def stream_matmul(a, st, w_t, nblk):
        N = st.buf.shape[1]
        kpc = st.chunk // 128
        for kt in range(st.n * kpc):
            a_s[kt] = a[:, kt * 128:(kt + 1) * 128]
        acc_s[:, 0:N] = jnp.zeros((2 * B, N), _F32)

        def body(i, carry):
            st.copy(i).wait()
            for u in range(kpc):
                kt = i * kpc + u
                a_k = a_s[kt]
                r = pl.multiple_of(kt * 128, 128)
                rh = pl.multiple_of(kt * 64, 64)
                for j in range(N // nblk):
                    w = st.buf[pl.ds(r, 128), j * nblk:(j + 1) * nblk]
                    w_t[pl.ds(rh, 64), j * nblk:(j + 1) * nblk] = (
                        pltpu.bitcast(w, jnp.uint32))
                    acc_s[:, j * nblk:(j + 1) * nblk] += _dot(a_k, w)
            return carry

        jax.lax.fori_loop(0, st.n, body, 0)
        return acc_s[:, 0:N]

    def wt(w_t, k0, k1, n0, n1):
        return pltpu.bitcast(w_t[k0 // 2:k1 // 2, n0:n1], _BF16)

    def put_q(q, h0):
        for h in range(q.shape[1] // Dh):
            q_s[(h0 + h) * B:(h0 + h + 1) * B, :] = q[:, h * Dh:(h + 1) * Dh]

    def scores(b, g, c):
        qg = q_s[pl.ds(g * rep * B + b, rep, stride=B), :].astype(_BF16)
        s = _dot(qg, pltpu.bitcast(kt_s[b, g], _BF16))
        m = jnp.max(s, axis=-1, keepdims=True)
        e = jnp.exp2((s - m) * c)
        l = jnp.sum(e, axis=-1, keepdims=True)
        return e.astype(_BF16), l

    def pv(b, g, e, l):
        o = _dot(e, v_s[b, g]) / l
        o_s[pl.ds(g * rep * B + b, rep, stride=B), :] = o

    def get_o(h0, h1):
        return jnp.concatenate(
            [o_s[h * B:(h + 1) * B, :] for h in range(h0, h1)], axis=1)

    m, _, r = _ln_stats(x)
    qq = stream_matmul(_with_ones(x), wq_st, wq_t, 1024)
    csq = qq[B:]
    put_q((qq[:B] - m * csq) * (r * scale), 0)

    def attn1(b, carry):
        kv_copy(b, 0).wait()
        for g in range(Hkv):
            kt_s[b, g] = pltpu.bitcast(k_s[b, g].T, jnp.uint32)
        el = [scores(b, g, _LOG2E) for g in range(Hkv)]
        kv_copy(b, 1).wait()
        for g in range(Hkv):
            pv(b, g, *el[g])
        return carry

    jax.lax.fori_loop(0, B, attn1, 0)
    x = x + stream_matmul(_with_ones(get_o(0, Hq)), wo_st, wo_t, 1024)[:B]
    x = x.astype(_BF16).astype(_F32)
    a, c = _ln2_coeffs(x)
    hh = stream_matmul(_with_ones(x), w1_st, w1_t, 896)
    cs1 = hh[B:]
    h32 = _gelu_tanh(a * hh[:B] - c * cs1 + b1)
    h = h32.astype(_BF16)
    x = x + b2 + stream_matmul(_with_ones(h32[:, :_R1]), w2_st, w2_t, 1024)[:B]

    acc = [x[:, j * 128:(j + 1) * 128] for j in range(NJ)]
    left = [F - _R1] * NJ
    xbs = [None] * NJ
    qpre = [None] * Hkv
    for (r0, r1, c0, c1), buf, cp, parts in zip(rects, rect_bufs, rect_cp, _QSCHED):
        cp.wait()
        if c1 - c0 == 128:
            acc[c0 // 128] = acc[c0 // 128] + _dot(h[:, r0:r1], buf[...])
        else:
            for kk in range(r0, r1, 128):
                w = buf[kk - r0:kk - r0 + 128, :]
                w2_t[kk // 2:(kk + 128) // 2, c0:c1] = pltpu.bitcast(w, jnp.uint32)
                d = _dot(h[:, kk:kk + 128], w)
                for j in range(c0 // 128, c1 // 128):
                    acc[j] = acc[j] + d[:, j * 128 - c0:(j + 1) * 128 - c0]
        for j in range(c0 // 128, c1 // 128):
            left[j] -= r1 - r0
            if left[j] == 0:
                xbs[j] = acc[j].astype(_BF16)
        for j, gs in parts:
            for g in gs:
                d = _dot(xbs[j], wt(wq_t, j * 128, (j + 1) * 128, g * G, (g + 1) * G))
                qpre[g] = d if qpre[g] is None else qpre[g] + d

    x = jnp.concatenate(xbs, axis=1).astype(_F32)
    m, _, r = _ln_stats(x)
    rs = r * (scale * _LOG2E)
    for g in range(Hkv):
        put_q(qpre[g] - m * csq[:, g * G:(g + 1) * G], g * rep)
    el = {}
    for g in range(Hkv):
        for b in range(B):
            el[b, g] = scores(b, g, rs[b:b + 1, :])
    for g in range(Hkv):
        for b in range(B):
            pv(b, g, *el[b, g])
    acc = x
    for g in range(Hkv):
        acc = acc + _dot(get_o(g * rep, (g + 1) * rep).astype(_BF16),
                         wt(wo_t, g * G, (g + 1) * G, 0, D))
    xb = acc.astype(_BF16)
    x = xb.astype(_F32)
    a, c = _ln2_coeffs(x)
    hp = None
    for j in range(NJ):
        d = _dot(xb[:, j * 128:(j + 1) * 128], wt(w1_t, j * 128, (j + 1) * 128, 0, F))
        hp = d if hp is None else hp + d
    h = _gelu_tanh(a * hp - c * cs1 + b1).astype(_BF16)
    acc = x + b2
    for f0 in range(0, _RA, 256):
        acc = acc + _dot(h[:, f0:f0 + 256], wt(w2_t, f0, f0 + 256, 0, D))
    h_tail = h[:, _RA:]
    acc = acc + jnp.concatenate(
        [_dot(h_tail, wt(w2_t, _RA, F, 0, D - 128)), _dot(h_tail, p7[...])], axis=1)

    o_ref[...] = acc.astype(o_ref.dtype)


@jax.jit
def pallas_interleave_layers__sliding_block_cached__mixer_channel_mlp__decode_kernel(
    A_x: jax.Array,
    A_k_cache: jax.Array,
    A_v_cache: jax.Array,
    A_wq: jax.Array,
    A_wo: jax.Array,
    B_x: jax.Array,
    B_w1: jax.Array,
    B_b1: jax.Array,
    B_w2: jax.Array,
    B_b2: jax.Array,
):
    del B_x
    B, Sq, D = A_x.shape
    _, Hkv, Sk, Dh = A_k_cache.shape
    Hq = A_wq.shape[1] // Dh
    F = B_w1.shape[1]
    W = min(4096, max(256, Sk // 4))
    assert (B, Sq, D, Hq, Hkv, Dh, F) == (8, 1, 1024, 32, 4, 128, 3584)

    kernel = functools.partial(
        _kernel, B=B, D=D, Hq=Hq, Hkv=Hkv, Sk=Sk, Dh=Dh, W=W, F=F)
    u32 = jnp.uint32
    scratch = [
        pltpu.VMEM((B, D), _BF16),
        pltpu.VMEM((F,), _BF16),
        pltpu.VMEM((D,), _BF16),
        pltpu.VMEM((B, Hkv, W, Dh), _BF16),
        pltpu.VMEM((B, Hkv, W, Dh), _BF16),
        pltpu.VMEM((B, Hkv, Dh // 2, W), u32),
        pltpu.VMEM((D, Hq * Dh), _BF16),
        pltpu.VMEM((Hq * Dh, D), _BF16),
        pltpu.VMEM((D, F), _BF16),
        pltpu.VMEM((_R1, D), _BF16),
        pltpu.VMEM((D // 2, Hq * Dh), u32),
        pltpu.VMEM((Hq * Dh // 2, D), u32),
        pltpu.VMEM((D // 2, F), u32),
        pltpu.VMEM((F // 2, D), u32),
        pltpu.VMEM((Hq * Dh // 128, 2 * B, 128), _BF16),
        pltpu.VMEM((2 * B, Hq * Dh), _F32),
        pltpu.VMEM(((Hq + 1) * B, Dh), _F32),
        pltpu.VMEM(((Hq + 1) * B, Dh), _F32),
    ] + [pltpu.VMEM((r1 - r0, c1 - c0), _BF16) for (r0, r1, c0, c1) in _w2_rects(F, D)]
    out = pl.pallas_call(
        kernel,
        out_shape=jax.ShapeDtypeStruct((B, D), A_x.dtype),
        in_specs=[pl.BlockSpec(memory_space=pl.ANY)] * 9,
        out_specs=pl.BlockSpec(memory_space=pltpu.VMEM),
        scratch_shapes=scratch,
        compiler_params=pltpu.CompilerParams(vmem_limit_bytes=110 * 1024 * 1024),
    )(A_x.reshape(B, D), A_k_cache, A_v_cache, A_wq, A_wo, B_w1, B_b1, B_w2, B_b2)
    return out.reshape(B, Sq, D)
```
